```python
import jax
import jax.numpy as jnp

def _softmax(x, axis=-1):
    return jax.nn.softmax(x, axis=axis)
def _gelu(x):
    return jax.nn.gelu(x, approximate=True)
def _silu(x):
    return jax.nn.silu(x)
def _sigmoid(x):
    return jax.nn.sigmoid(x)
def _layernorm(x, axis=-1, eps=1e-5):
    m = jnp.mean(x, axis=axis, keepdims=True)
    v = jnp.var(x, axis=axis, keepdims=True)
    return (x - m) / jnp.sqrt(v + eps)
def _scatter_add(tgt, idx, src, axis=0):
    return tgt.at[idx].add(src)
def _segment_sum(src, seg, n):
    return jax.ops.segment_sum(src, seg, n)
class _Rng:
    def __init__(self, key):
        self._k = key
    def _next(self):
        self._k, sub = jax.random.split(self._k)
        return sub
    def normal(self, shape):
        return jax.random.normal(self._next(), shape, dtype=jnp.bfloat16)
    def randint(self, lo, hi, shape):
        return jax.random.randint(self._next(), shape, lo, hi, dtype=jnp.int32)
    def uniform(self, shape, lo=0.0, hi=1.0):
        return jax.random.uniform(self._next(), shape, jnp.bfloat16, lo, hi)
    def permutation(self, n):
        return jax.random.permutation(self._next(), n)


kernel_name = 'parallel_sum__compressed_kv_cla__geglu_ffn__decode'

def _fwd_setup_inputs():
    _rng = _Rng(jax.random.key(int.from_bytes(__import__("os").urandom(4), "little")))
    _w = (lambda a: (lambda t: t.astype(jnp.bfloat16) if jnp.issubdtype(t.dtype, jnp.floating) else t)(jnp.asarray(a)))
    def _A_setup():
        B, H, Sq, Sk, D, M = 8, 32, 1, 4096, 128, 512
        Dc = 4 * D
        return {
            "x": _w((lambda *s: _rng.normal(s) * 0.05)(B, Sq, M)),
            "c_kv": _w((lambda *s: _rng.normal(s) * 0.05)(B, Sk, Dc)),
            "w_q": _w((lambda *s: _rng.normal(s) * 0.05)(M, H, D) * (M ** -0.5)),
            "w_uk": _w((lambda *s: _rng.normal(s) * 0.05)(Dc, H, D) * (Dc ** -0.5)),
            "w_uv": _w((lambda *s: _rng.normal(s) * 0.05)(Dc, H, D) * (Dc ** -0.5)),
            "w_o": _w((lambda *s: _rng.normal(s) * 0.05)(H, D, M) * ((H * D) ** -0.5)),
        }
    _A_in = _A_setup()

    def _B_setup():
        B, S, D, F = 8, 1, 512, 1376
        return {
            "x": _w((lambda *s: _rng.normal(s) * 0.05)(B, S, D)),
            "w_gate": _w((lambda *s: _rng.normal(s) * 0.05)(D, F)),
            "w_up": _w((lambda *s: _rng.normal(s) * 0.05)(D, F)),
            "w_down": _w((lambda *s: _rng.normal(s) * 0.05)(F, D)),
        }
    _B_in = _B_setup()

    return {
        "A_x": _A_in["x"],
        "A_c_kv": _A_in["c_kv"],
        "A_w_q": _A_in["w_q"],
        "A_w_uk": _A_in["w_uk"],
        "A_w_uv": _A_in["w_uv"],
        "A_w_o": _A_in["w_o"],
        "B_x": _B_in["x"],
        "B_w_gate": _B_in["w_gate"],
        "B_w_up": _B_in["w_up"],
        "B_w_down": _B_in["w_down"],
    }

def _fwd_reference(A_x, A_c_kv, A_w_q, A_w_uk, A_w_uv, A_w_o, B_x, B_w_gate, B_w_up, B_w_down):
    def _A_ref(x, c_kv, w_q, w_uk, w_uv, w_o):
        B, Sq, M = x.shape[0], x.shape[1], x.shape[2]
        Sk = c_kv.shape[1]
        H, D = w_q.shape[1], w_q.shape[2]
        q = jnp.einsum("bqm,mhd->bhqd", x, w_q)
        k = jnp.einsum("bkc,chd->bhkd", c_kv, w_uk)
        v = jnp.einsum("bkc,chd->bhkd", c_kv, w_uv)
        scores = jnp.einsum("bhqd,bhkd->bhqk", q, k) * (D ** -0.5)
        off = Sk - Sq
        qi = jnp.arange(Sq)[:, None]
        kj = jnp.arange(Sk)[None, :]
        cmask = kj <= (qi + off)
        scores = jnp.where(cmask[None, None], scores, -1e9)
        p = _softmax(scores, axis=-1)
        ctx = jnp.einsum("bhqk,bhkd->bhqd", p, v)
        return jnp.einsum("bhqd,hdm->bqm", ctx, w_o)

    def _B_ref(x, w_gate, w_up, w_down):
        return (_gelu(x @ w_gate) * (x @ w_up)) @ w_down

    x = A_x
    xn = _layernorm(x, axis=-1)
    return x + _A_ref(xn, A_c_kv, A_w_q, A_w_uk, A_w_uv, A_w_o) + _B_ref(xn, B_w_gate, B_w_up, B_w_down)


def setup_inputs():
    _inp = _fwd_setup_inputs()
    _gk = jax.random.fold_in(jax.random.key(int.from_bytes(__import__("os").urandom(4), "little")), 2**31 - 1)
    _shapes = [[8, 1, 512]]
    _dtypes = ['bfloat16']
    _gks = jax.random.split(_gk, len(_shapes))
    _gs = [jax.random.normal(k, s, dtype=jnp.dtype(d)) * 0.05 for k, s, d in zip(_gks, _shapes, _dtypes)]
    _inp["grad_out"] = _gs[0]
    return _inp

def reference(A_x, A_c_kv, A_w_q, A_w_uk, A_w_uv, A_w_o, B_w_gate, B_w_up, B_w_down, B_x, grad_out):
    _const = dict(B_x=B_x)
    def _f(*_d):
        return _fwd_reference(**{'A_x': _d[0], 'A_c_kv': _d[1], 'A_w_q': _d[2], 'A_w_uk': _d[3], 'A_w_uv': _d[4], 'A_w_o': _d[5], 'B_w_gate': _d[6], 'B_w_up': _d[7], 'B_w_down': _d[8], **_const})
    _out, _vjp = jax.vjp(_f, A_x, A_c_kv, A_w_q, A_w_uk, A_w_uv, A_w_o, B_w_gate, B_w_up, B_w_down)
    _grads = _vjp(grad_out)
    _out0 = jnp.asarray(_out)
    return (_out0, *[jnp.asarray(_g) for _g in _grads])
```

```python
import functools
import math
import jax
import jax.numpy as jnp
from jax import lax
from jax.experimental import pallas as pl
from jax.experimental.pallas import tpu as pltpu

_BF = jnp.bfloat16
_F32 = jnp.float32
_NN = (((1,), (0,)), ((), ()))
_NT = (((1,), (1,)), ((), ()))
_TN = (((0,), (0,)), ((), ()))
_BNN = (((2,), (1,)), ((0,), (0,)))
_BNT = (((2,), (2,)), ((0,), (0,)))


def _dot(a, b, dims):
    return lax.dot_general(a, b, dims, preferred_element_type=_F32)


def _make_kernel(B, SK, M, H, D, DC, F, cfg):
    scale = float(D) ** -0.5
    eps = 1e-5
    G = 16
    NG = H // G
    WRITE_AT = cfg.get("write_at", 6)
    SWAP_CH = cfg.get("swap_ch", 32)
    GR_CH = cfg.get("gr_ch", 64)

    def kernel(x_hbm, ckv_hbm, wq_hbm, wuk_hbm, wuv_hbm, wo_hbm, wg_hbm, wu_hbm, wd_hbm, g_hbm,
               out_hbm, dx_hbm, dckv_hbm, dwq_hbm, dwuk_hbm, dwuv_hbm, dwo_hbm, dwg_hbm, dwu_hbm, dwd_hbm,
               x_v, g_v, c_v, d_v, wq_v, wuk_v, wuv_v, wo_v, wq_s, wuk_s, wuv_s, dwo_v,
               wg_v, wu_v, wd_v, dwg_v, dwu_v, dwd_v, out_v, dx_v,
               q_v, dctx_v, wall_v, oall_v, s_v, p_v, rsem, wsem):
        def rd(src, dst, i):
            return pltpu.make_async_copy(src, dst, rsem.at[i])

        r_x = rd(x_hbm, x_v, 0)
        r_g = rd(g_hbm, g_v, 1)
        r_wq = rd(wq_hbm, wq_v, 2)
        r_wuk = rd(wuk_hbm, wuk_v, 3)
        r_wo = rd(wo_hbm, wo_v, 4)
        r_wuv = rd(wuv_hbm, wuv_v, 5)
        r_wg = rd(wg_hbm, wg_v, 6)
        r_wu = rd(wu_hbm, wu_v, 7)
        r_wd = rd(wd_hbm, wd_v, 8)

        def r_c(b):
            return rd(ckv_hbm.at[b], c_v.at[b], 9 + b)

        def wr(src, dst, i):
            return pltpu.make_async_copy(src, dst, wsem.at[i])

        def w_d(b):
            return wr(d_v.at[b], dckv_hbm.at[b], 9 + b)

        w_out = wr(out_v, out_hbm, 0)
        w_dx = wr(dx_v, dx_hbm, 1)
        w_dwq = wr(wq_v, dwq_hbm, 2)
        w_dwuk = wr(wuk_v, dwuk_hbm, 3)
        w_dwo = wr(dwo_v, dwo_hbm, 4)
        w_dwuv = wr(wuv_v, dwuv_hbm, 5)
        w_dwg = wr(dwg_v, dwg_hbm, 6)
        w_dwu = wr(dwu_v, dwu_hbm, 7)
        w_dwd = wr(dwd_v, dwd_hbm, 8)

        for r in (r_x, r_g, r_wq, r_wuk, r_wo, r_wuv):
            r.start()
        for b in range(B):
            r_c(b).start()
        for r in (r_wg, r_wu, r_wd):
            r.start()

        def swap(src, dst):
            def body(i, c):
                sl = pl.ds(pl.multiple_of(i * SWAP_CH, SWAP_CH), SWAP_CH)
                dst[:, sl, :] = jnp.swapaxes(src[sl], 0, 1)
                return c
            lax.fori_loop(0, src.shape[0] // SWAP_CH, body, 0)

        with jax.named_scope("prologue"):
            r_x.wait()
            r_g.wait()
            x = x_v[...].astype(_F32)
            g32 = g_v[...].astype(_F32)
            g = g32.astype(_BF)
            mu = jnp.mean(x, axis=-1, keepdims=True)
            xc = x - mu
            var = jnp.mean(xc * xc, axis=-1, keepdims=True)
            rstd = lax.rsqrt(var + eps)
            xn32 = xc * rstd
            xn = xn32.astype(_BF)

            r_wq.wait()
            swap(wq_v, wq_s)
            q = _dot(jnp.broadcast_to(xn[None], (H, B, M)), wq_s[...], _BNN)
            q_v[...] = q
            r_wuk.wait()
            swap(wuk_v, wuk_s)
            qa = _dot(q.astype(_BF), wuk_s[...], _BNT)
            wall_v[:, 0:H, :] = jnp.swapaxes(qa, 0, 1).astype(_BF)
            r_wo.wait()
            dctx = _dot(jnp.broadcast_to(g[None], (H, B, M)), wo_v[...], _BNT)
            dctx_v[...] = dctx
            r_wuv.wait()
            swap(wuv_v, wuv_s)
            dcc = _dot(dctx.astype(_BF), wuv_s[...], _BNT)
            wall_v[:, H:2 * H, :] = jnp.swapaxes(dcc, 0, 1).astype(_BF)

        def batch(b, carry):
            r_c(b).wait()
            wb = wall_v[b]
            s_v[...] = _dot(wb, c_v[b], _NT)

            @pl.when(b == WRITE_AT)
            def _():
                r_wg.wait()
                r_wu.wait()
                r_wd.wait()
                for bb in range(WRITE_AT):
                    w_d(bb).start()

            s = s_v[0:H, :]
            m = jnp.max(s, axis=1, keepdims=True)
            e = jnp.exp((s - m) * scale)
            l = jnp.sum(e, axis=1, keepdims=True)
            dp = s_v[H:2 * H, :]
            rl = 1.0 / l
            delta = jnp.sum(e * dp, axis=1, keepdims=True) * rl
            p = e * rl
            ds = p * ((dp - delta) * scale)
            p_v[0:H, :] = ds.astype(_BF)
            p_v[H:2 * H, :] = p.astype(_BF)
            p2 = p_v[...]
            oall_v[b] = _dot(p2, c_v[b], _NN)
            d_v[b] = _dot(p2, wb, _TN).astype(_BF)

            @pl.when(b >= WRITE_AT)
            def _():
                w_d(b).start()
            return carry

        with jax.named_scope("attention"):
            lax.fori_loop(0, B, batch, 0)

        with jax.named_scope("ffn"):
            a = _dot(xn, wg_v[...], _NT)
            u = _dot(xn, wu_v[...], _NT)
            k0 = math.sqrt(2.0 / math.pi)
            k1 = 0.044715
            th = jnp.tanh(k0 * (a + k1 * a * a * a))
            ga = 0.5 * a * (1.0 + th)
            dga = 0.5 * (1.0 + th) + 0.5 * a * (1.0 - th * th) * (k0 * (1.0 + 3.0 * k1 * a * a))
            hh = (ga * u).astype(_BF)
            ffn = _dot(hh, wd_v[...], _NN)
            dh = _dot(g, wd_v[...], _NT)
            da = (dh * u * dga).astype(_BF)
            du = (dh * ga).astype(_BF)
            dxn = _dot(da, wg_v[...], _NN) + _dot(du, wu_v[...], _NN)
            dwg_v[...] = _dot(da, xn, _TN).astype(_BF)
            w_dwg.start()
            dwu_v[...] = _dot(du, xn, _TN).astype(_BF)
            w_dwu.start()
            dwd_v[...] = _dot(hh, g, _TN).astype(_BF)
            w_dwd.start()

        row = lax.broadcasted_iota(jnp.int32, (G, B * G), 0)
        lane = lax.broadcasted_iota(jnp.int32, (G, B * G), 1)
        diag = (lane % G) == row

        def delta_grad(a_g, y_g, dst, g0):
            at = a_g.T
            n = at.shape[0]
            for c0 in range(0, n, GR_CH):
                blk = at[c0:c0 + GR_CH]
                lhs = jnp.where(diag[None], blk[:, None, :], 0.0).astype(_BF).reshape(GR_CH * G, B * G)
                o = _dot(lhs, y_g, _NN).astype(_BF)
                dst[c0:c0 + GR_CH, g0:g0 + G, :] = o.reshape(GR_CH, G, D)

        with jax.named_scope("epi_uk"):
            qb = jnp.swapaxes(q_v[...], 0, 1)
            for gi in range(NG):
                a_g = oall_v[:, gi * G:(gi + 1) * G, :].reshape(B * G, DC)
                y_g = qb[:, gi * G:(gi + 1) * G, :].reshape(B * G, D).astype(_BF)
                delta_grad(a_g, y_g, wuk_v, gi * G)
            w_dwuk.start()
        with jax.named_scope("epi_uv"):
            db = jnp.swapaxes(dctx_v[...], 0, 1)
            for gi in range(NG):
                a_g = oall_v[:, H + gi * G:H + (gi + 1) * G, :].reshape(B * G, DC)
                y_g = db[:, gi * G:(gi + 1) * G, :].reshape(B * G, D).astype(_BF)
                delta_grad(a_g, y_g, wuv_v, gi * G)
            w_dwuv.start()
        with jax.named_scope("epi_o"):
            ot = jnp.swapaxes(oall_v[...], 0, 1).astype(_BF)
            ctx = _dot(ot[H:2 * H], wuv_s[...], _BNN)
            ctxb = ctx.astype(_BF)
            attn = jnp.sum(_dot(ctxb, wo_v[...], _BNN), axis=0)
            ctx2 = jnp.swapaxes(ctxb, 0, 1).reshape(B, H * D)
            dwo_v[...] = _dot(ctx2, g, _TN).astype(_BF).reshape(H, D, M)
            w_dwo.start()
        with jax.named_scope("epi_q"):
            dq = _dot(ot[0:H], wuk_s[...], _BNN)
            dqb = dq.astype(_BF)
            dxn = dxn + jnp.sum(_dot(dqb, wq_s[...], _BNT), axis=0)
            dqs = jnp.swapaxes(dq, 0, 1)
            a_x = jnp.broadcast_to(xn.astype(_F32)[:, None, :], (B, G, M)).reshape(B * G, M)
            for gi in range(NG):
                y_g = dqs[:, gi * G:(gi + 1) * G, :].reshape(B * G, D).astype(_BF)
                delta_grad(a_x, y_g, wq_v, gi * G)
            w_dwq.start()
        with jax.named_scope("final"):
            out = x + attn + ffn
            out_v[...] = out.astype(_BF)
            w_out.start()
            m1 = jnp.mean(dxn, axis=-1, keepdims=True)
            m2 = jnp.mean(dxn * xn32, axis=-1, keepdims=True)
            dx = g32 + rstd * (dxn - m1 - xn32 * m2)
            dx_v[...] = dx.astype(_BF)
            w_dx.start()
            for b in range(B):
                w_d(b).wait()
            for w in (w_dwg, w_dwu, w_dwd, w_dwuk, w_dwuv, w_dwo, w_dwq, w_out, w_dx):
                w.wait()

    return kernel


_CFG = {}


@jax.jit
def pallas_parallel_sum__compressed_kv_cla__geglu_ffn__decode_kernel(
    A_x, A_c_kv, A_w_q, A_w_uk, A_w_uv, A_w_o, B_x, B_w_gate, B_w_up, B_w_down, grad_out,
):
    cfg = _CFG

    B, _, M = A_x.shape
    SK, DC = A_c_kv.shape[1:]
    H, D = A_w_q.shape[1:]
    F = B_w_gate.shape[1]
    bf = _BF
    x2 = A_x.reshape(B, M)
    g2 = grad_out.reshape(B, M)
    wgT = B_w_gate.T
    wuT = B_w_up.T
    ins = (x2, A_c_kv, A_w_q, A_w_uk, A_w_uv, A_w_o, wgT, wuT, B_w_down, g2)
    outs = (x2, x2, A_c_kv, A_w_q, A_w_uk, A_w_uv, A_w_o, wgT, wuT, B_w_down)
    any_spec = pl.BlockSpec(memory_space=pl.ANY)
    V = pltpu.VMEM
    scratch = [
        V((B, M), bf), V((B, M), bf),
        V((B, SK, DC), bf), V((B, SK, DC), bf),
        V((M, H, D), bf), V((DC, H, D), bf), V((DC, H, D), bf), V((H, D, M), bf),
        V((H, M, D), bf), V((H, DC, D), bf), V((H, DC, D), bf),
        V((H, D, M), bf),
        V((F, M), bf), V((F, M), bf), V((F, M), bf),
        V((F, M), bf), V((F, M), bf), V((F, M), bf),
        V((B, M), bf), V((B, M), bf),
        V((H, B, D), _F32), V((H, B, D), _F32),
        V((B, 2 * H, DC), bf), V((B, 2 * H, DC), _F32),
        V((2 * H, SK), _F32), V((2 * H, SK), bf),
        pltpu.SemaphoreType.DMA((9 + B,)), pltpu.SemaphoreType.DMA((9 + B,)),
    ]
    res = pl.pallas_call(
        _make_kernel(B, SK, M, H, D, DC, F, cfg),
        out_shape=tuple(jax.ShapeDtypeStruct(o.shape, o.dtype) for o in outs),
        in_specs=[any_spec] * len(ins),
        out_specs=tuple([any_spec] * len(outs)),
        scratch_shapes=scratch,
        compiler_params=pltpu.CompilerParams(vmem_limit_bytes=128 * 1024 * 1024),
        name="mla_ffn_fwd_bwd",
    )(*ins)
    out, dx, dckv, dwq, dwuk, dwuv, dwo, dwgT, dwuT, dwd = res
    return (out.reshape(B, 1, M), dx.reshape(B, 1, M), dckv, dwq, dwuk, dwuv, dwo, dwgT.T, dwuT.T, dwd)
```

```python
import math

import jax
import jax.numpy as jnp
from jax import lax
from jax.experimental import pallas as pl
from jax.experimental.pallas import tpu as pltpu

_BF = jnp.bfloat16
_F32 = jnp.float32
_NN = (((1,), (0,)), ((), ()))
_NT = (((1,), (1,)), ((), ()))
_TN = (((0,), (0,)), ((), ()))
_BNN = (((2,), (1,)), ((0,), (0,)))
_BNT = (((2,), (2,)), ((0,), (0,)))

_EPS = 1e-5
_HG = 16
_SWAP_CH = 32
_N_SEM = 4
_SYNC_BATCH = 6
_D_REGIONS = 4
_D_GROUP = 2
_D_ISSUE = (-1, 6, 7, 7)
_W_REGIONS = 8
_F_REGIONS = 2
_SEG_ROWS = 16
_SEG_LAT = 2
_TAIL_ROWS = 480


def _dot(a, b, dims):
    return lax.dot_general(a, b, dims, preferred_element_type=_F32)


def _make_kernel(B, SK, M, H, D, DC, F):
    scale = float(D) ** -0.5
    n_hg = H // _HG
    d_rows = SK // _D_REGIONS
    w_lat = M // _W_REGIONS
    o_rows = H * D // _W_REGIONS
    f_rows = F // _F_REGIONS
    n_grp = B // _D_GROUP
    first_c, ffn_head, ffn_tail = 4, 4 + B, 5 + B
    sem_w = ffn_head % _N_SEM

    def kernel(x_hbm, ckv_hbm, wq_hbm, wuk_hbm, wuv_hbm, wo_hbm, wg_hbm, wu_hbm, wd_hbm, g_hbm,
               out_hbm, dx_hbm, dckv_hbm, dwq_hbm, dwuk_hbm, dwuv_hbm, dwo_hbm, dwg_hbm, dwu_hbm, dwd_hbm,
               x_v, g_v, c_v, d_v, wq_v, wuk_v, wuv_v, wo_v, wq_s, wuk_s, wuv_s, dwo_v,
               wg_v, wu_v, wd_v, dwg_v, dwu_v, dwd_v, out_v, dx_v,
               q_v, dctx_v, wall_v, oall_v, s_v, p_v, sem):

        def cp(src, dst, i):
            return pltpu.make_async_copy(src, dst, sem.at[i])

        def r_c(b):
            return cp(ckv_hbm.at[b], c_v.at[b], (first_c + b) % _N_SEM)

        def item(i):
            s = i % _N_SEM
            if i == 0:
                return [cp(wq_hbm, wq_v, s), cp(x_hbm, x_v, s), cp(g_hbm, g_v, s)]
            if i == 1:
                return [cp(wuk_hbm, wuk_v, s)]
            if i == 2:
                return [cp(wo_hbm, wo_v, s)]
            if i == 3:
                return [cp(wuv_hbm, wuv_v, s)]
            if i < ffn_head:
                return [r_c(i - first_c)]
            head, tail = pl.ds(0, F - _TAIL_ROWS), pl.ds(F - _TAIL_ROWS, _TAIL_ROWS)
            if i == ffn_head:
                return [cp(wg_hbm, wg_v, s), cp(wu_hbm, wu_v, s), cp(wd_hbm.at[head], wd_v.at[head], s)]
            return [cp(wd_hbm.at[tail], wd_v.at[tail], s)]

        def start_item(i):
            for d in item(i):
                d.start()

        def wait_item(i):
            for d in item(i):
                d.wait()

        def pieces(pairs, lead, n, seg):
            assert n % seg == 0

            def run(act):
                def body(j, carry):
                    sl = pl.ds(pl.multiple_of(j * seg, seg), seg)
                    for src, dst in pairs:
                        act(cp(src.at[lead, sl], dst.at[lead, sl], sem_w))
                    return carry
                lax.fori_loop(0, n // seg, body, 0)

            return (lambda: run(lambda d: d.start())), (lambda: run(lambda d: d.wait()))

        every = slice(None)
        per_grp = _D_GROUP * _D_REGIONS
        w_d = [pieces([(d_v, dckv_hbm)], pl.ds(i * per_grp, per_grp), d_rows, _SEG_ROWS) for i in range(n_grp)]
        w_dwuk = pieces([(wuk_v, dwuk_hbm)], every, w_lat, _SEG_LAT)
        w_dwuv = pieces([(wuv_v, dwuv_hbm)], every, w_lat, _SEG_LAT)
        w_dwo = pieces([(dwo_v, dwo_hbm)], every, o_rows, _SEG_ROWS)
        w_dwq = pieces([(wq_v, dwq_hbm)], every, w_lat, _SEG_LAT)
        w_dffn = pieces([(dwg_v, dwg_hbm), (dwu_v, dwu_hbm), (dwd_v, dwd_hbm)], every, f_rows, _SEG_ROWS)
        w_out = cp(out_v, out_hbm, sem_w)
        w_dx = cp(dx_v, dx_hbm, sem_w)

        for i in range(_N_SEM):
            start_item(i)

        def to_head_major(src, dst):
            per = w_lat // _SWAP_CH

            def body(i, carry):
                blk = src[i // per, pl.ds(pl.multiple_of((i % per) * _SWAP_CH, _SWAP_CH), _SWAP_CH)]
                dst[:, pl.ds(pl.multiple_of(i * _SWAP_CH, _SWAP_CH), _SWAP_CH), :] = jnp.swapaxes(blk, 0, 1)
                return carry
            lax.fori_loop(0, _W_REGIONS * per, body, 0)

        wait_item(0)
        start_item(_N_SEM)
        x = x_v[...].astype(_F32)
        g = g_v[...]
        xc = x - jnp.mean(x, axis=-1, keepdims=True)
        rstd = lax.rsqrt(jnp.mean(xc * xc, axis=-1, keepdims=True) + _EPS)
        xn32 = xc * rstd
        xn = xn32.astype(_BF)

        to_head_major(wq_v, wq_s)
        q = _dot(jnp.broadcast_to(xn[None], (H, B, M)), wq_s[...], _BNN)
        q_v[...] = q
        wait_item(1)
        start_item(1 + _N_SEM)
        to_head_major(wuk_v, wuk_s)
        qa = _dot(q.astype(_BF), wuk_s[...], _BNT)
        wall_v[:, 0:H, :] = jnp.swapaxes(qa, 0, 1).astype(_BF)
        wait_item(2)
        start_item(2 + _N_SEM)
        dctx = _dot(jnp.broadcast_to(g[None], (H, B, M)), wo_v[...], _BNT)
        dctx_v[...] = dctx
        wait_item(3)
        start_item(3 + _N_SEM)
        to_head_major(wuv_v, wuv_s)
        dcc = _dot(dctx.astype(_BF), wuv_s[...], _BNT)
        wall_v[:, H:2 * H, :] = jnp.swapaxes(dcc, 0, 1).astype(_BF)

        def batch(b, carry):
            r_c(b).wait()

            @pl.when(b + _N_SEM < B)
            def _():
                r_c(b + _N_SEM).start()

            @pl.when(b + _N_SEM == B)
            def _():
                start_item(ffn_head)

            @pl.when(b + _N_SEM == B + 1)
            def _():
                start_item(ffn_tail)

            wb = wall_v[b]
            s_v[...] = _dot(wb, c_v[b], _NT)

            @pl.when(b == _SYNC_BATCH)
            def _():
                wait_item(ffn_head)
                for i in range(n_grp):
                    if _D_ISSUE[i] < 0:
                        w_d[i][0]()

            s = s_v[0:H, :]
            e = jnp.exp((s - jnp.max(s, axis=1, keepdims=True)) * scale)
            rl = 1.0 / jnp.sum(e, axis=1, keepdims=True)
            dp = s_v[H:2 * H, :]
            delta = jnp.sum(e * dp, axis=1, keepdims=True) * rl
            p = e * rl
            p_v[0:H, :] = (p * ((dp - delta) * scale)).astype(_BF)
            p_v[H:2 * H, :] = p.astype(_BF)
            p2 = p_v[...]
            oall_v[b] = _dot(p2, c_v[b], _NN)
            d_v[pl.ds(b * _D_REGIONS, _D_REGIONS)] = (
                _dot(p2, wb, _TN).astype(_BF).reshape(_D_REGIONS, d_rows, DC))

            for i in range(n_grp):
                if _D_ISSUE[i] >= 0:
                    @pl.when(b == _D_ISSUE[i])
                    def _(i=i):
                        w_d[i][0]()
            return carry

        lax.fori_loop(0, B, batch, 0)

        diag = (lax.broadcasted_iota(jnp.int32, (_HG, B * _HG), 1) % _HG
                == lax.broadcasted_iota(jnp.int32, (_HG, B * _HG), 0))

        def head_grad(a_g, y_g, dst, h0):
            at = a_g.T
            for r in range(_W_REGIONS):
                blk = at[r * w_lat:(r + 1) * w_lat]
                lhs = jnp.where(diag[None], blk[:, None, :], 0.0).astype(_BF).reshape(w_lat * _HG, B * _HG)
                dst[r, :, h0:h0 + _HG, :] = _dot(lhs, y_g, _NN).astype(_BF).reshape(w_lat, _HG, D)

        def group(y_bhd, h0):
            return y_bhd[:, h0:h0 + _HG, :].reshape(B * _HG, D).astype(_BF)

        qb = jnp.swapaxes(q_v[...], 0, 1)
        for i in range(n_hg):
            h0 = i * _HG
            head_grad(oall_v[:, h0:h0 + _HG, :].reshape(B * _HG, DC), group(qb, h0), wuk_v, h0)
        w_dwuk[0]()

        db = jnp.swapaxes(dctx_v[...], 0, 1)
        for i in range(n_hg):
            h0 = i * _HG
            head_grad(oall_v[:, H + h0:H + h0 + _HG, :].reshape(B * _HG, DC), group(db, h0), wuv_v, h0)
        w_dwuv[0]()

        ot = jnp.swapaxes(oall_v[...], 0, 1).astype(_BF)
        ctx = _dot(ot[H:2 * H], wuv_s[...], _BNN).astype(_BF)
        attn = jnp.sum(_dot(ctx, wo_v[...], _BNN), axis=0)
        ctx2 = jnp.swapaxes(ctx, 0, 1).reshape(B, H * D)
        dwo_v[...] = _dot(ctx2, g, _TN).astype(_BF).reshape(_W_REGIONS, o_rows, M)
        w_dwo[0]()

        dq = _dot(ot[0:H], wuk_s[...], _BNN)
        dxn_attn = jnp.sum(_dot(dq.astype(_BF), wq_s[...], _BNT), axis=0)
        dqb = jnp.swapaxes(dq, 0, 1)
        xn_rep = jnp.broadcast_to(xn.astype(_F32)[:, None, :], (B, _HG, M)).reshape(B * _HG, M)
        for i in range(n_hg):
            head_grad(xn_rep, group(dqb, i * _HG), wq_v, i * _HG)
        w_dwq[0]()

        wait_item(ffn_tail)
        a = _dot(xn, wg_v[...], _NT)
        u = _dot(xn, wu_v[...], _NT)
        k0, k1 = math.sqrt(2.0 / math.pi), 0.044715
        th = jnp.tanh(k0 * (a + k1 * a * a * a))
        gelu = 0.5 * a * (1.0 + th)
        dgelu = 0.5 * (1.0 + th) + 0.5 * a * (1.0 - th * th) * (k0 * (1.0 + 3.0 * k1 * a * a))
        hh = (gelu * u).astype(_BF)
        ffn = _dot(hh, wd_v[...], _NN)
        dh = _dot(g, wd_v[...], _NT)
        da = (dh * u * dgelu).astype(_BF)
        du = (dh * gelu).astype(_BF)
        out_v[...] = (x + attn + ffn).astype(_BF)
        w_out.start()
        dxn = dxn_attn + _dot(da, wg_v[...], _NN) + _dot(du, wu_v[...], _NN)
        m1 = jnp.mean(dxn, axis=-1, keepdims=True)
        m2 = jnp.mean(dxn * xn32, axis=-1, keepdims=True)
        dx_v[...] = (g.astype(_F32) + rstd * (dxn - m1 - xn32 * m2)).astype(_BF)
        w_dx.start()
        dwg_v[...] = _dot(da, xn, _TN).astype(_BF).reshape(_F_REGIONS, f_rows, M)
        dwu_v[...] = _dot(du, xn, _TN).astype(_BF).reshape(_F_REGIONS, f_rows, M)
        dwd_v[...] = _dot(hh, g, _TN).astype(_BF).reshape(_F_REGIONS, f_rows, M)
        w_dffn[0]()

        for w in w_d + [w_dwuk, w_dwuv, w_dwo, w_dwq]:
            w[1]()
        w_out.wait()
        w_dx.wait()
        w_dffn[1]()

    return kernel


@jax.jit
def pallas_parallel_sum__compressed_kv_cla__geglu_ffn__decode_kernel(
    A_x, A_c_kv, A_w_q, A_w_uk, A_w_uv, A_w_o, B_x, B_w_gate, B_w_up, B_w_down, grad_out,
):
    del B_x
    B, _, M = A_x.shape
    SK, DC = A_c_kv.shape[1:]
    H, D = A_w_q.shape[1:]
    F = B_w_gate.shape[1]
    assert DC == M and B == len(_D_ISSUE) * _D_GROUP and H % _HG == 0
    bf = _BF

    w4 = (_W_REGIONS, M // _W_REGIONS, H, D)
    d3 = (B * _D_REGIONS, SK // _D_REGIONS, DC)
    o3 = (_W_REGIONS, H * D // _W_REGIONS, M)
    f3 = (_F_REGIONS, F // _F_REGIONS, M)
    ins = (A_x.reshape(B, M), A_c_kv, A_w_q.reshape(w4), A_w_uk.reshape(w4), A_w_uv.reshape(w4), A_w_o,
           B_w_gate.T, B_w_up.T, B_w_down, grad_out.reshape(B, M))
    out_shapes = ((B, M), (B, M), d3, w4, w4, w4, o3, f3, f3, f3)

    hbm = pl.BlockSpec(memory_space=pl.ANY)
    vmem = pltpu.VMEM
    scratch = [
        vmem((B, M), bf), vmem((B, M), bf),
        vmem((B, SK, DC), bf), vmem(d3, bf),
        vmem(w4, bf), vmem(w4, bf), vmem(w4, bf), vmem((H, D, M), bf),
        vmem((H, M, D), bf), vmem((H, DC, D), bf), vmem((H, DC, D), bf),
        vmem(o3, bf),
        vmem((F, M), bf), vmem((F, M), bf), vmem((F, M), bf),
        vmem(f3, bf), vmem(f3, bf), vmem(f3, bf),
        vmem((B, M), bf), vmem((B, M), bf),
        vmem((H, B, D), _F32), vmem((H, B, D), _F32),
        vmem((B, 2 * H, DC), bf), vmem((B, 2 * H, DC), _F32),
        vmem((2 * H, SK), _F32), vmem((2 * H, SK), bf),
        pltpu.SemaphoreType.DMA((_N_SEM,)),
    ]
    out, dx, dckv, dwq, dwuk, dwuv, dwo, dwg_t, dwu_t, dwd = pl.pallas_call(
        _make_kernel(B, SK, M, H, D, DC, F),
        out_shape=tuple(jax.ShapeDtypeStruct(s, bf) for s in out_shapes),
        in_specs=[hbm] * len(ins),
        out_specs=tuple([hbm] * len(out_shapes)),
        scratch_shapes=scratch,
        compiler_params=pltpu.CompilerParams(vmem_limit_bytes=128 * 1024 * 1024),
        name="mla_ffn_fwd_bwd",
    )(*ins)
    return (out.reshape(B, 1, M), dx.reshape(B, 1, M), dckv.reshape(B, SK, DC), dwq.reshape(M, H, D),
            dwuk.reshape(DC, H, D), dwuv.reshape(DC, H, D), dwo.reshape(H, D, M),
            dwg_t.reshape(F, M).T, dwu_t.reshape(F, M).T, dwd.reshape(F, M))
```

```python
import math

import jax
import jax.numpy as jnp
from jax import lax
from jax.experimental import pallas as pl
from jax.experimental.pallas import tpu as pltpu

_BF = jnp.bfloat16
_F32 = jnp.float32
_NN = (((1,), (0,)), ((), ()))
_NT = (((1,), (1,)), ((), ()))
_TN = (((0,), (0,)), ((), ()))
_BNN = (((2,), (1,)), ((0,), (0,)))
_BNT = (((2,), (2,)), ((0,), (0,)))

_EPS = 1e-5
_HG = 16
_SWAP_CH = 32
_HEAD_STEPS = 8

_N_SEM = 8
_N_PACED = 10
_N_PIECES = 16
_SPIN = 50
_TAIL_ROWS = 480

_D_REGIONS = 4
_D_GROUP = 2
_W_REGIONS = 8
_F_REGIONS = 2
_SEG_ROWS = 16
_SEG_LAT = 2
_SYNC_BATCH = 2
_D_SYNC = 64
_D_PLAN = ((3, 100), (4, 128), (5, 173), (6, 192), (7, 256))


def _dot(a, b, dims):
    return lax.dot_general(a, b, dims, preferred_element_type=_F32)


def _make_kernel(B, SK, M, H, D, DC, F):
    scale = float(D) ** -0.5
    n_hg = H // _HG
    hs = H // _HEAD_STEPS
    d_rows = SK // _D_REGIONS
    w_lat = M // _W_REGIONS
    o_rows = H * D // _W_REGIONS
    f_rows = F // _F_REGIONS
    d_lead = _D_GROUP * _D_REGIONS
    d_per_grp = d_rows // _SEG_ROWS
    d_total = B // _D_GROUP * d_per_grp
    first_c, ffn_head, ffn_tail = 4, 4 + B, 5 + B
    sem_w = ffn_head % _N_SEM
    assert first_c < _N_PACED <= ffn_head and B <= _N_SEM < first_c + B + 1
    assert _D_SYNC <= (_SYNC_BATCH + 1) // _D_GROUP * d_per_grp and _D_PLAN[-1][1] == d_total
    assert all(n <= (k + 1) // _D_GROUP * d_per_grp for k, n in _D_PLAN)

    def kernel(x_hbm, ckv_hbm, wq_hbm, wuk_hbm, wuv_hbm, wo_hbm, wg_hbm, wu_hbm, wd_hbm, g_hbm,
               out_hbm, dx_hbm, dckv_hbm, dwq_hbm, dwuk_hbm, dwuv_hbm, dwo_hbm, dwg_hbm, dwu_hbm, dwd_hbm,
               x_v, g_v, c_v, d_v, wq_v, wuk_v, wuv_v, wo_v, wq_s, wuk_s, wuv_s, dwo_v,
               wg_v, wu_v, wd_v, dwg_v, dwu_v, dwd_v, out_v, dx_v,
               q_v, dctx_v, wall_v, oall_v, s_v, p_v, t_v, spin_v, sem):

        def cp(src, dst, i):
            return pltpu.make_async_copy(src, dst, sem.at[i])

        weights = {0: (wq_hbm, wq_v), 1: (wuk_hbm, wuk_v), 2: (wo_hbm, wo_v), 3: (wuv_hbm, wuv_v)}

        def part(i, lo, n):
            if i < first_c:
                src, dst = weights[i]
                if i == 2:
                    st = H // (2 * _N_PIECES)
                    sl = (pl.ds(lo * st, n * st),)
                else:
                    st = w_lat // (2 * _N_PIECES)
                    sl = (slice(None), pl.ds(lo * st, n * st))
            else:
                src, dst = ckv_hbm, c_v
                st = SK // (2 * _N_PIECES)
                sl = (i - first_c, pl.ds(pl.multiple_of(lo * st, st), n * st))
            return cp(src.at[sl], dst.at[sl], i % _N_SEM)

        def activations():
            return [cp(x_hbm, x_v, 0), cp(g_hbm, g_v, 0)]

        def r_c(b):
            return cp(ckv_hbm.at[b], c_v.at[b], (first_c + b) % _N_SEM)

        def whole(i):
            s = i % _N_SEM
            if i < first_c:
                return [cp(weights[i][0], weights[i][1], s)]
            if i < ffn_head:
                return [r_c(i - first_c)]
            hd, tail = pl.ds(0, F - _TAIL_ROWS), pl.ds(F - _TAIL_ROWS, _TAIL_ROWS)
            if i == ffn_head:
                return [cp(wg_hbm, wg_v, s), cp(wu_hbm, wu_v, s), cp(wd_hbm.at[hd], wd_v.at[hd], s)]
            return [cp(wd_hbm.at[tail], wd_v.at[tail], s)]

        def start_item(i):
            for d in ([part(i, 0, _N_PIECES)] if i < _N_PACED else whole(i)):
                d.start(priority=1)

        def wait_item(i):
            for d in whole(i):
                d.wait()

        def tick(i, j):
            part(i, _N_PIECES + j, 1).start(priority=0)

        def idle_ticks(i, j0):
            def body(j, acc):
                tick(i, j)
                return lax.fori_loop(0, _SPIN, lambda k, c: c * 1.0001 + 1.0, acc)
            if j0 < _N_PIECES:
                spin_v[...] = lax.fori_loop(j0, _N_PIECES, body, jnp.zeros((8, 128), _F32))

        def pieces(pairs, n, seg):
            assert n % seg == 0

            def run(act):
                def body(j, carry):
                    sl = pl.ds(pl.multiple_of(j * seg, seg), seg)
                    for src, dst in pairs:
                        act(cp(src.at[:, sl], dst.at[:, sl], sem_w))
                    return carry
                lax.fori_loop(0, n // seg, body, 0)

            return (lambda: run(lambda d: d.start())), (lambda: run(lambda d: d.wait()))

        def d_copy(grp, j):
            lead = pl.ds(grp * d_lead, d_lead)
            sl = pl.ds(j * _SEG_ROWS, _SEG_ROWS)
            return cp(d_v.at[lead, sl], dckv_hbm.at[lead, sl], sem_w)

        def start_d(lo, hi):
            for k in range(lo, hi):
                d_copy(k // d_per_grp, k % d_per_grp).start()

        w_dwuk = pieces([(wuk_v, dwuk_hbm)], w_lat, _SEG_LAT)
        w_dwuv = pieces([(wuv_v, dwuv_hbm)], w_lat, _SEG_LAT)
        w_dwo = pieces([(dwo_v, dwo_hbm)], o_rows, _SEG_ROWS)
        w_dwq = pieces([(wq_v, dwq_hbm)], w_lat, _SEG_LAT)
        w_dffn = pieces([(dwg_v, dwg_hbm), (dwu_v, dwu_hbm), (dwd_v, dwd_hbm)], f_rows, _SEG_ROWS)
        w_out = cp(out_v, out_hbm, sem_w)
        w_dx = cp(dx_v, dx_hbm, sem_w)

        def to_head_major(src, dst, it):
            per = w_lat // _SWAP_CH
            steps = _W_REGIONS * per // 2

            def body(i2, carry):
                tick(it, i2)
                for u in range(2):
                    i = 2 * i2 + u
                    blk = src[i // per, pl.ds(pl.multiple_of((i % per) * _SWAP_CH, _SWAP_CH), _SWAP_CH)]
                    dst[:, pl.ds(pl.multiple_of(i * _SWAP_CH, _SWAP_CH), _SWAP_CH), :] = jnp.swapaxes(blk, 0, 1)
                return carry
            lax.fori_loop(0, steps, body, 0)
            return steps

        def per_head(lhs, w_ref, dims, dst, it, j0):
            def body(i, carry):
                tick(it, j0 + i)
                sl = pl.ds(i * hs, hs)
                dst[sl] = _dot(lhs(sl), w_ref[sl], dims)
                return carry
            lax.fori_loop(0, _HEAD_STEPS, body, 0)
            return j0 + _HEAD_STEPS

        for d in activations():
            d.start(priority=0)
        for i in range(_N_SEM):
            start_item(i)

        idle_ticks(0, 0)
        for d in activations():
            d.wait()
        wait_item(0)
        start_item(_N_SEM)
        x = x_v[...].astype(_F32)
        g = g_v[...]
        xc = x - jnp.mean(x, axis=-1, keepdims=True)
        rstd = lax.rsqrt(jnp.mean(xc * xc, axis=-1, keepdims=True) + _EPS)
        xn32 = xc * rstd
        xn = xn32.astype(_BF)
        xn_h = jnp.broadcast_to(xn[None], (hs, B, M))
        g_h = jnp.broadcast_to(g[None], (hs, B, M))

        j = to_head_major(wq_v, wq_s, 1)
        idle_ticks(1, per_head(lambda sl: xn_h, wq_s, _BNN, q_v, 1, j))
        wait_item(1)
        start_item(1 + _N_SEM)
        j = to_head_major(wuk_v, wuk_s, 2)
        j = per_head(lambda sl: q_v[sl].astype(_BF), wuk_s, _BNT, t_v, 2, j)
        wall_v[:, 0:H, :] = jnp.swapaxes(t_v[...], 0, 1).astype(_BF)
        idle_ticks(2, j)
        wait_item(2)
        start_item(2 + _N_SEM)
        idle_ticks(3, per_head(lambda sl: g_h, wo_v, _BNT, dctx_v, 3, 0))
        wait_item(3)
        start_item(3 + _N_SEM)
        j = to_head_major(wuv_v, wuv_s, 4)
        j = per_head(lambda sl: dctx_v[sl].astype(_BF), wuv_s, _BNT, t_v, 4, j)
        wall_v[:, H:2 * H, :] = jnp.swapaxes(t_v[...], 0, 1).astype(_BF)
        idle_ticks(4, j)
        for i in range(5, _N_PACED):
            idle_ticks(i, 0)

        def batch(b, carry):
            r_c(b).wait()

            if _N_SEM < B:
                @pl.when(b + _N_SEM < B)
                def _():
                    r_c(b + _N_SEM).start(priority=1)

            @pl.when(b + _N_SEM == B)
            def _():
                start_item(ffn_head)

            @pl.when(b + _N_SEM == B + 1)
            def _():
                start_item(ffn_tail)

            wb = wall_v[b]
            s_v[...] = _dot(wb, c_v[b], _NT)
            s = s_v[0:H, :]
            e = jnp.exp((s - jnp.max(s, axis=1, keepdims=True)) * scale)
            rl = 1.0 / jnp.sum(e, axis=1, keepdims=True)
            dp = s_v[H:2 * H, :]
            delta = jnp.sum(e * dp, axis=1, keepdims=True) * rl
            p = e * rl
            p_v[0:H, :] = (p * ((dp - delta) * scale)).astype(_BF)
            p_v[H:2 * H, :] = p.astype(_BF)
            p2 = p_v[...]
            oall_v[b] = _dot(p2, c_v[b], _NN)
            d_v[pl.ds(b * _D_REGIONS, _D_REGIONS)] = (
                _dot(p2, wb, _TN).astype(_BF).reshape(_D_REGIONS, d_rows, DC))

            @pl.when(b == _SYNC_BATCH)
            def _():
                wait_item(ffn_head)
                start_d(0, _D_SYNC)

            lo = _D_SYNC
            for k, hi in _D_PLAN:
                @pl.when(b == k)
                def _(lo=lo, hi=hi):
                    start_d(lo, hi)
                lo = hi
            return carry

        lax.fori_loop(0, B, batch, 0)

        diag = (lax.broadcasted_iota(jnp.int32, (_HG, B * _HG), 1) % _HG
                == lax.broadcasted_iota(jnp.int32, (_HG, B * _HG), 0))

        def head_grad(a_g, y_g, dst, h0):
            at = a_g.T
            for r in range(_W_REGIONS):
                blk = at[r * w_lat:(r + 1) * w_lat]
                lhs = jnp.where(diag[None], blk[:, None, :], 0.0).astype(_BF).reshape(w_lat * _HG, B * _HG)
                dst[r, :, h0:h0 + _HG, :] = _dot(lhs, y_g, _NN).astype(_BF).reshape(w_lat, _HG, D)

        def group(y_bhd, h0):
            return y_bhd[:, h0:h0 + _HG, :].reshape(B * _HG, D).astype(_BF)

        qb = jnp.swapaxes(q_v[...], 0, 1)
        for i in range(n_hg):
            h0 = i * _HG
            head_grad(oall_v[:, h0:h0 + _HG, :].reshape(B * _HG, DC), group(qb, h0), wuk_v, h0)
        w_dwuk[0]()

        db = jnp.swapaxes(dctx_v[...], 0, 1)
        for i in range(n_hg):
            h0 = i * _HG
            head_grad(oall_v[:, H + h0:H + h0 + _HG, :].reshape(B * _HG, DC), group(db, h0), wuv_v, h0)
        w_dwuv[0]()

        ot = jnp.swapaxes(oall_v[...], 0, 1).astype(_BF)
        ctx = _dot(ot[H:2 * H], wuv_s[...], _BNN).astype(_BF)
        attn = jnp.sum(_dot(ctx, wo_v[...], _BNN), axis=0)
        ctx2 = jnp.swapaxes(ctx, 0, 1).reshape(B, H * D)
        dwo_v[...] = _dot(ctx2, g, _TN).astype(_BF).reshape(_W_REGIONS, o_rows, M)
        w_dwo[0]()

        dq = _dot(ot[0:H], wuk_s[...], _BNN)
        dxn_attn = jnp.sum(_dot(dq.astype(_BF), wq_s[...], _BNT), axis=0)
        dqb = jnp.swapaxes(dq, 0, 1)
        xn_rep = jnp.broadcast_to(xn.astype(_F32)[:, None, :], (B, _HG, M)).reshape(B * _HG, M)
        for i in range(n_hg):
            head_grad(xn_rep, group(dqb, i * _HG), wq_v, i * _HG)
        w_dwq[0]()

        wait_item(ffn_tail)
        a = _dot(xn, wg_v[...], _NT)
        u = _dot(xn, wu_v[...], _NT)
        k0, k1 = math.sqrt(2.0 / math.pi), 0.044715
        th = jnp.tanh(k0 * (a + k1 * a * a * a))
        gelu = 0.5 * a * (1.0 + th)
        dgelu = 0.5 * (1.0 + th) + 0.5 * a * (1.0 - th * th) * (k0 * (1.0 + 3.0 * k1 * a * a))
        hh = (gelu * u).astype(_BF)
        ffn = _dot(hh, wd_v[...], _NN)
        dh = _dot(g, wd_v[...], _NT)
        da = (dh * u * dgelu).astype(_BF)
        du = (dh * gelu).astype(_BF)
        out_v[...] = (x + attn + ffn).astype(_BF)
        w_out.start()
        dxn = dxn_attn + _dot(da, wg_v[...], _NN) + _dot(du, wu_v[...], _NN)
        m1 = jnp.mean(dxn, axis=-1, keepdims=True)
        m2 = jnp.mean(dxn * xn32, axis=-1, keepdims=True)
        dx_v[...] = (g.astype(_F32) + rstd * (dxn - m1 - xn32 * m2)).astype(_BF)
        w_dx.start()
        dwg_v[...] = _dot(da, xn, _TN).astype(_BF).reshape(_F_REGIONS, f_rows, M)
        dwu_v[...] = _dot(du, xn, _TN).astype(_BF).reshape(_F_REGIONS, f_rows, M)
        dwd_v[...] = _dot(hh, g, _TN).astype(_BF).reshape(_F_REGIONS, f_rows, M)
        w_dffn[0]()

        def wait_d(k, carry):
            lead = pl.ds((k // d_per_grp) * d_lead, d_lead)
            sl = pl.ds(pl.multiple_of((k % d_per_grp) * _SEG_ROWS, _SEG_ROWS), _SEG_ROWS)
            cp(d_v.at[lead, sl], dckv_hbm.at[lead, sl], sem_w).wait()
            return carry
        lax.fori_loop(0, d_total, wait_d, 0)
        for w in (w_dwuk, w_dwuv, w_dwo, w_dwq):
            w[1]()
        w_out.wait()
        w_dx.wait()
        w_dffn[1]()

    return kernel


@jax.jit
def pallas_parallel_sum__compressed_kv_cla__geglu_ffn__decode_kernel(
    A_x, A_c_kv, A_w_q, A_w_uk, A_w_uv, A_w_o, B_x, B_w_gate, B_w_up, B_w_down, grad_out,
):
    del B_x
    B, _, M = A_x.shape
    SK, DC = A_c_kv.shape[1:]
    H, D = A_w_q.shape[1:]
    F = B_w_gate.shape[1]
    assert DC == M and H % _HG == 0
    bf = _BF

    w4 = (_W_REGIONS, M // _W_REGIONS, H, D)
    d3 = (B * _D_REGIONS, SK // _D_REGIONS, DC)
    o3 = (_W_REGIONS, H * D // _W_REGIONS, M)
    f3 = (_F_REGIONS, F // _F_REGIONS, M)
    ins = (A_x.reshape(B, M), A_c_kv, A_w_q.reshape(w4), A_w_uk.reshape(w4), A_w_uv.reshape(w4), A_w_o,
           B_w_gate.T, B_w_up.T, B_w_down, grad_out.reshape(B, M))
    out_shapes = ((B, M), (B, M), d3, w4, w4, w4, o3, f3, f3, f3)

    hbm = pl.BlockSpec(memory_space=pl.ANY)
    vmem = pltpu.VMEM
    scratch = [
        vmem((B, M), bf), vmem((B, M), bf),
        vmem((B, SK, DC), bf), vmem(d3, bf),
        vmem(w4, bf), vmem(w4, bf), vmem(w4, bf), vmem((H, D, M), bf),
        vmem((H, M, D), bf), vmem((H, DC, D), bf), vmem((H, DC, D), bf),
        vmem(o3, bf),
        vmem((F, M), bf), vmem((F, M), bf), vmem((F, M), bf),
        vmem(f3, bf), vmem(f3, bf), vmem(f3, bf),
        vmem((B, M), bf), vmem((B, M), bf),
        vmem((H, B, D), _F32), vmem((H, B, D), _F32),
        vmem((B, 2 * H, DC), bf), vmem((B, 2 * H, DC), _F32),
        vmem((2 * H, SK), _F32), vmem((2 * H, SK), bf),
        vmem((H, B, DC), _F32), vmem((8, 128), _F32),
        pltpu.SemaphoreType.DMA((_N_SEM,)),
    ]
    out, dx, dckv, dwq, dwuk, dwuv, dwo, dwg_t, dwu_t, dwd = pl.pallas_call(
        _make_kernel(B, SK, M, H, D, DC, F),
        out_shape=tuple(jax.ShapeDtypeStruct(s, bf) for s in out_shapes),
        in_specs=[hbm] * len(ins),
        out_specs=tuple([hbm] * len(out_shapes)),
        scratch_shapes=scratch,
        compiler_params=pltpu.CompilerParams(vmem_limit_bytes=128 * 1024 * 1024),
        name="mla_ffn_fwd_bwd",
    )(*ins)
    return (out.reshape(B, 1, M), dx.reshape(B, 1, M), dckv.reshape(B, SK, DC), dwq.reshape(M, H, D),
            dwuk.reshape(DC, H, D), dwuv.reshape(DC, H, D), dwo.reshape(H, D, M),
            dwg_t.reshape(F, M).T, dwu_t.reshape(F, M).T, dwd.reshape(F, M))
```

```python
import math

import jax
import jax.numpy as jnp
from jax import lax
from jax.experimental import pallas as pl
from jax.experimental.pallas import tpu as pltpu

_BF = jnp.bfloat16
_F32 = jnp.float32
_NN = (((1,), (0,)), ((), ()))
_NT = (((1,), (1,)), ((), ()))
_TN = (((0,), (0,)), ((), ()))
_BNN = (((2,), (1,)), ((0,), (0,)))
_BNT = (((2,), (2,)), ((0,), (0,)))

_EPS = 1e-5
_HG = 16
_SWAP_CH = 32
_HEAD_STEPS = 8

_N_SEM = 8
_N_PACED = 10
_N_PIECES = 16
_SPIN = 50
_TAIL_ROWS = 480

_D_REGIONS = 4
_D_GROUP = 2
_W_REGIONS = 8
_F_REGIONS = 2
_SEG_ROWS = 16
_SEG_LAT = 2
_SYNC_BATCH = 2
_D_SYNC = 64
_D_PLAN = ((3, 100), (4, 128), (5, 173), (6, 192), (7, 256))


def _dot(a, b, dims):
    return lax.dot_general(a, b, dims, preferred_element_type=_F32)


def _make_kernel(B, SK, M, H, D, DC, F):
    scale = float(D) ** -0.5
    n_hg = H // _HG
    hs = H // _HEAD_STEPS
    d_rows = SK // _D_REGIONS
    w_lat = M // _W_REGIONS
    o_rows = H * D // _W_REGIONS
    f_rows = F // _F_REGIONS
    d_lead = _D_GROUP * _D_REGIONS
    d_per_grp = d_rows // _SEG_ROWS
    d_total = B // _D_GROUP * d_per_grp
    first_c, ffn_head, ffn_tail = 4, 4 + B, 5 + B
    sem_w = ffn_head % _N_SEM
    assert first_c < _N_PACED <= ffn_head and B <= _N_SEM < first_c + B + 1
    assert _D_SYNC <= (_SYNC_BATCH + 1) // _D_GROUP * d_per_grp and _D_PLAN[-1][1] == d_total
    assert all(n <= (k + 1) // _D_GROUP * d_per_grp for k, n in _D_PLAN)

    def kernel(x_hbm, ckv_hbm, wq_hbm, wuk_hbm, wuv_hbm, wo_hbm, wg_hbm, wu_hbm, wd_hbm, g_hbm,
               out_hbm, dx_hbm, dckv_hbm, dwq_hbm, dwuk_hbm, dwuv_hbm, dwo_hbm, dwg_hbm, dwu_hbm, dwd_hbm,
               x_v, g_v, c_v, d_v, wq_v, wuk_v, wuv_v, wo_v, wq_s, wuk_s, wuv_s, dwo_v,
               wg_v, wu_v, wd_v, dwg_v, dwu_v, dwd_v, out_v, dx_v,
               q_v, dctx_v, wall_v, oall_v, s_v, p_v, t_v, spin_v, sem):

        def cp(src, dst, i):
            return pltpu.make_async_copy(src, dst, sem.at[i])

        weights = {0: (wq_hbm, wq_v), 1: (wuk_hbm, wuk_v), 2: (wo_hbm, wo_v), 3: (wuv_hbm, wuv_v)}

        def part(i, lo, n):
            if i < first_c:
                src, dst = weights[i]
                if i == 2:
                    st = H // (2 * _N_PIECES)
                    sl = (pl.ds(lo * st, n * st),)
                else:
                    st = w_lat // (2 * _N_PIECES)
                    sl = (slice(None), pl.ds(lo * st, n * st))
            else:
                src, dst = ckv_hbm, c_v
                st = SK // (2 * _N_PIECES)
                sl = (i - first_c, pl.ds(pl.multiple_of(lo * st, st), n * st))
            return cp(src.at[sl], dst.at[sl], i % _N_SEM)

        def activations():
            return [cp(x_hbm, x_v, 0), cp(g_hbm, g_v, 0)]

        def r_c(b):
            return cp(ckv_hbm.at[b], c_v.at[b], (first_c + b) % _N_SEM)

        def whole(i):
            s = i % _N_SEM
            if i < first_c:
                return [cp(weights[i][0], weights[i][1], s)]
            if i < ffn_head:
                return [r_c(i - first_c)]
            hd, tail = pl.ds(0, F - _TAIL_ROWS), pl.ds(F - _TAIL_ROWS, _TAIL_ROWS)
            if i == ffn_head:
                return [cp(wg_hbm, wg_v, s), cp(wu_hbm, wu_v, s), cp(wd_hbm.at[hd], wd_v.at[hd], s)]
            return [cp(wd_hbm.at[tail], wd_v.at[tail], s)]

        def start_item(i):
            for d in ([part(i, 0, _N_PIECES)] if i < _N_PACED else whole(i)):
                d.start(priority=1)

        def wait_item(i):
            for d in whole(i):
                d.wait()

        def tick(i, j):
            part(i, _N_PIECES + j, 1).start(priority=0)

        def idle_ticks(i, j0):
            def body(j, acc):
                tick(i, j)
                return lax.fori_loop(0, _SPIN, lambda k, c: c * 1.0001 + 1.0, acc)
            if j0 < _N_PIECES:
                spin_v[...] = lax.fori_loop(j0, _N_PIECES, body, jnp.zeros((8, 128), _F32))

        def start_pieces(pairs, n, seg):
            assert n % seg == 0

            def body(j, carry):
                sl = pl.ds(pl.multiple_of(j * seg, seg), seg)
                for src, dst in pairs:
                    cp(src.at[:, sl], dst.at[:, sl], sem_w).start()
                return carry
            lax.fori_loop(0, n // seg, body, 0)

        def start_d(lo, hi):
            for k in range(lo, hi):
                lead = pl.ds(k // d_per_grp * d_lead, d_lead)
                sl = pl.ds(k % d_per_grp * _SEG_ROWS, _SEG_ROWS)
                cp(d_v.at[lead, sl], dckv_hbm.at[lead, sl], sem_w).start()

        def to_head_major(src, dst, it):
            per = w_lat // _SWAP_CH
            steps = _W_REGIONS * per // 2

            def body(i2, carry):
                tick(it, i2)
                for u in range(2):
                    i = 2 * i2 + u
                    blk = src[i // per, pl.ds(pl.multiple_of((i % per) * _SWAP_CH, _SWAP_CH), _SWAP_CH)]
                    dst[:, pl.ds(pl.multiple_of(i * _SWAP_CH, _SWAP_CH), _SWAP_CH), :] = jnp.swapaxes(blk, 0, 1)
                return carry
            lax.fori_loop(0, steps, body, 0)
            return steps

        def per_head(lhs, w_ref, dims, dst, it, j0):
            def body(i, carry):
                tick(it, j0 + i)
                sl = pl.ds(i * hs, hs)
                dst[sl] = _dot(lhs(sl), w_ref[sl], dims)
                return carry
            lax.fori_loop(0, _HEAD_STEPS, body, 0)
            return j0 + _HEAD_STEPS

        for d in activations():
            d.start(priority=0)
        for i in range(_N_SEM):
            start_item(i)

        idle_ticks(0, 0)
        for d in activations():
            d.wait()
        wait_item(0)
        start_item(_N_SEM)
        x = x_v[...].astype(_F32)
        g = g_v[...]
        xc = x - jnp.mean(x, axis=-1, keepdims=True)
        rstd = lax.rsqrt(jnp.mean(xc * xc, axis=-1, keepdims=True) + _EPS)
        xn32 = xc * rstd
        xn = xn32.astype(_BF)
        xn_h = jnp.broadcast_to(xn[None], (hs, B, M))
        g_h = jnp.broadcast_to(g[None], (hs, B, M))

        j = to_head_major(wq_v, wq_s, 1)
        idle_ticks(1, per_head(lambda sl: xn_h, wq_s, _BNN, q_v, 1, j))
        wait_item(1)
        start_item(1 + _N_SEM)
        j = to_head_major(wuk_v, wuk_s, 2)
        j = per_head(lambda sl: q_v[sl].astype(_BF), wuk_s, _BNT, t_v, 2, j)
        wall_v[:, 0:H, :] = jnp.swapaxes(t_v[...], 0, 1).astype(_BF)
        idle_ticks(2, j)
        wait_item(2)
        start_item(2 + _N_SEM)
        idle_ticks(3, per_head(lambda sl: g_h, wo_v, _BNT, dctx_v, 3, 0))
        wait_item(3)
        start_item(3 + _N_SEM)
        j = to_head_major(wuv_v, wuv_s, 4)
        j = per_head(lambda sl: dctx_v[sl].astype(_BF), wuv_s, _BNT, t_v, 4, j)
        wall_v[:, H:2 * H, :] = jnp.swapaxes(t_v[...], 0, 1).astype(_BF)
        idle_ticks(4, j)
        for i in range(5, _N_PACED):
            idle_ticks(i, 0)

        def batch(b, carry):
            r_c(b).wait()

            if _N_SEM < B:
                @pl.when(b + _N_SEM < B)
                def _():
                    r_c(b + _N_SEM).start(priority=1)

            @pl.when(b + _N_SEM == B)
            def _():
                start_item(ffn_head)

            @pl.when(b + _N_SEM == B + 1)
            def _():
                start_item(ffn_tail)

            wb = wall_v[b]
            s_v[...] = _dot(wb, c_v[b], _NT)
            s = s_v[0:H, :]
            e = jnp.exp((s - jnp.max(s, axis=1, keepdims=True)) * scale)
            rl = 1.0 / jnp.sum(e, axis=1, keepdims=True)
            dp = s_v[H:2 * H, :]
            delta = jnp.sum(e * dp, axis=1, keepdims=True) * rl
            p = e * rl
            p_v[0:H, :] = (p * ((dp - delta) * scale)).astype(_BF)
            p_v[H:2 * H, :] = p.astype(_BF)
            p2 = p_v[...]
            oall_v[b] = _dot(p2, c_v[b], _NN)
            d_v[pl.ds(b * _D_REGIONS, _D_REGIONS)] = (
                _dot(p2, wb, _TN).astype(_BF).reshape(_D_REGIONS, d_rows, DC))

            @pl.when(b == _SYNC_BATCH)
            def _():
                wait_item(ffn_head)
                start_d(0, _D_SYNC)

            lo = _D_SYNC
            for k, hi in _D_PLAN:
                @pl.when(b == k)
                def _(lo=lo, hi=hi):
                    start_d(lo, hi)
                lo = hi
            return carry

        lax.fori_loop(0, B, batch, 0)

        diag = (lax.broadcasted_iota(jnp.int32, (_HG, B * _HG), 1) % _HG
                == lax.broadcasted_iota(jnp.int32, (_HG, B * _HG), 0))

        def head_grad(a_g, y_g, dst, h0):
            at = a_g.T
            for r in range(_W_REGIONS):
                blk = at[r * w_lat:(r + 1) * w_lat]
                lhs = jnp.where(diag[None], blk[:, None, :], 0.0).astype(_BF).reshape(w_lat * _HG, B * _HG)
                dst[r, :, h0:h0 + _HG, :] = _dot(lhs, y_g, _NN).astype(_BF).reshape(w_lat, _HG, D)

        def group(y_bhd, h0):
            return y_bhd[:, h0:h0 + _HG, :].reshape(B * _HG, D).astype(_BF)

        qb = jnp.swapaxes(q_v[...], 0, 1)
        for i in range(n_hg):
            h0 = i * _HG
            head_grad(oall_v[:, h0:h0 + _HG, :].reshape(B * _HG, DC), group(qb, h0), wuk_v, h0)
        start_pieces([(wuk_v, dwuk_hbm)], w_lat, _SEG_LAT)

        db = jnp.swapaxes(dctx_v[...], 0, 1)
        for i in range(n_hg):
            h0 = i * _HG
            head_grad(oall_v[:, H + h0:H + h0 + _HG, :].reshape(B * _HG, DC), group(db, h0), wuv_v, h0)
        start_pieces([(wuv_v, dwuv_hbm)], w_lat, _SEG_LAT)

        ot = jnp.swapaxes(oall_v[...], 0, 1).astype(_BF)
        ctx = _dot(ot[H:2 * H], wuv_s[...], _BNN).astype(_BF)
        attn = jnp.sum(_dot(ctx, wo_v[...], _BNN), axis=0)
        ctx2 = jnp.swapaxes(ctx, 0, 1).reshape(B, H * D)
        dwo_v[...] = _dot(ctx2, g, _TN).astype(_BF).reshape(_W_REGIONS, o_rows, M)
        start_pieces([(dwo_v, dwo_hbm)], o_rows, _SEG_ROWS)

        dq = _dot(ot[0:H], wuk_s[...], _BNN)
        dxn_attn = jnp.sum(_dot(dq.astype(_BF), wq_s[...], _BNT), axis=0)
        dqb = jnp.swapaxes(dq, 0, 1)
        xn_rep = jnp.broadcast_to(xn.astype(_F32)[:, None, :], (B, _HG, M)).reshape(B * _HG, M)
        for i in range(n_hg):
            head_grad(xn_rep, group(dqb, i * _HG), wq_v, i * _HG)
        start_pieces([(wq_v, dwq_hbm)], w_lat, _SEG_LAT)

        wait_item(ffn_tail)
        a = _dot(xn, wg_v[...], _NT)
        u = _dot(xn, wu_v[...], _NT)
        k0, k1 = math.sqrt(2.0 / math.pi), 0.044715
        th = jnp.tanh(k0 * (a + k1 * a * a * a))
        gelu = 0.5 * a * (1.0 + th)
        dgelu = 0.5 * (1.0 + th) + 0.5 * a * (1.0 - th * th) * (k0 * (1.0 + 3.0 * k1 * a * a))
        hh = (gelu * u).astype(_BF)
        ffn = _dot(hh, wd_v[...], _NN)
        dh = _dot(g, wd_v[...], _NT)
        da = (dh * u * dgelu).astype(_BF)
        du = (dh * gelu).astype(_BF)
        out_v[...] = (x + attn + ffn).astype(_BF)
        cp(out_v, out_hbm, sem_w).start()
        dxn = dxn_attn + _dot(da, wg_v[...], _NN) + _dot(du, wu_v[...], _NN)
        m1 = jnp.mean(dxn, axis=-1, keepdims=True)
        m2 = jnp.mean(dxn * xn32, axis=-1, keepdims=True)
        dx_v[...] = (g.astype(_F32) + rstd * (dxn - m1 - xn32 * m2)).astype(_BF)
        cp(dx_v, dx_hbm, sem_w).start()
        dwg_v[...] = _dot(da, xn, _TN).astype(_BF).reshape(_F_REGIONS, f_rows, M)
        dwu_v[...] = _dot(du, xn, _TN).astype(_BF).reshape(_F_REGIONS, f_rows, M)
        dwd_v[...] = _dot(hh, g, _TN).astype(_BF).reshape(_F_REGIONS, f_rows, M)
        start_pieces([(dwg_v, dwg_hbm), (dwu_v, dwu_hbm), (dwd_v, dwd_hbm)], f_rows, _SEG_ROWS)

        for src, dst in ((d_v, dckv_hbm), (wuk_v, dwuk_hbm), (wuv_v, dwuv_hbm), (dwo_v, dwo_hbm),
                         (wq_v, dwq_hbm), (out_v, out_hbm), (dx_v, dx_hbm), (dwg_v, dwg_hbm),
                         (dwu_v, dwu_hbm), (dwd_v, dwd_hbm)):
            cp(src, dst, sem_w).wait()

    return kernel


@jax.jit
def pallas_parallel_sum__compressed_kv_cla__geglu_ffn__decode_kernel(
    A_x, A_c_kv, A_w_q, A_w_uk, A_w_uv, A_w_o, B_x, B_w_gate, B_w_up, B_w_down, grad_out,
):
    del B_x
    B, _, M = A_x.shape
    SK, DC = A_c_kv.shape[1:]
    H, D = A_w_q.shape[1:]
    F = B_w_gate.shape[1]
    assert DC == M and H % _HG == 0
    bf = _BF

    w4 = (_W_REGIONS, M // _W_REGIONS, H, D)
    d3 = (B * _D_REGIONS, SK // _D_REGIONS, DC)
    o3 = (_W_REGIONS, H * D // _W_REGIONS, M)
    f3 = (_F_REGIONS, F // _F_REGIONS, M)
    ins = (A_x.reshape(B, M), A_c_kv, A_w_q.reshape(w4), A_w_uk.reshape(w4), A_w_uv.reshape(w4), A_w_o,
           B_w_gate.T, B_w_up.T, B_w_down, grad_out.reshape(B, M))
    out_shapes = ((B, M), (B, M), d3, w4, w4, w4, o3, f3, f3, f3)

    hbm = pl.BlockSpec(memory_space=pl.ANY)
    vmem = pltpu.VMEM
    scratch = [
        vmem((B, M), bf), vmem((B, M), bf),
        vmem((B, SK, DC), bf), vmem(d3, bf),
        vmem(w4, bf), vmem(w4, bf), vmem(w4, bf), vmem((H, D, M), bf),
        vmem((H, M, D), bf), vmem((H, DC, D), bf), vmem((H, DC, D), bf),
        vmem(o3, bf),
        vmem((F, M), bf), vmem((F, M), bf), vmem((F, M), bf),
        vmem(f3, bf), vmem(f3, bf), vmem(f3, bf),
        vmem((B, M), bf), vmem((B, M), bf),
        vmem((H, B, D), _F32), vmem((H, B, D), _F32),
        vmem((B, 2 * H, DC), bf), vmem((B, 2 * H, DC), _F32),
        vmem((2 * H, SK), _F32), vmem((2 * H, SK), bf),
        vmem((H, B, DC), _F32), vmem((8, 128), _F32),
        pltpu.SemaphoreType.DMA((_N_SEM,)),
    ]
    out, dx, dckv, dwq, dwuk, dwuv, dwo, dwg_t, dwu_t, dwd = pl.pallas_call(
        _make_kernel(B, SK, M, H, D, DC, F),
        out_shape=tuple(jax.ShapeDtypeStruct(s, bf) for s in out_shapes),
        in_specs=[hbm] * len(ins),
        out_specs=tuple([hbm] * len(out_shapes)),
        scratch_shapes=scratch,
        compiler_params=pltpu.CompilerParams(vmem_limit_bytes=128 * 1024 * 1024),
        name="mla_ffn_fwd_bwd",
    )(*ins)
    return (out.reshape(B, 1, M), dx.reshape(B, 1, M), dckv.reshape(B, SK, DC), dwq.reshape(M, H, D),
            dwuk.reshape(DC, H, D), dwuv.reshape(DC, H, D), dwo.reshape(H, D, M),
            dwg_t.reshape(F, M).T, dwu_t.reshape(F, M).T, dwd.reshape(F, M))
```

```python
import math

import jax
import jax.numpy as jnp
from jax import lax
from jax.experimental import pallas as pl
from jax.experimental.pallas import tpu as pltpu

_BF = jnp.bfloat16
_F32 = jnp.float32
_NN = (((1,), (0,)), ((), ()))
_NT = (((1,), (1,)), ((), ()))
_TN = (((0,), (0,)), ((), ()))
_BNN = (((2,), (1,)), ((0,), (0,)))
_BNT = (((2,), (2,)), ((0,), (0,)))

_EPS = 1e-5
_HG = 16
_SWAP_CH = 32
_HEAD_STEPS = 8

_N_SEM = 3
_N_PACED = 10
_N_PIECES = 16
_SPIN = 50
_TAIL_ROWS = 480

_D_REGIONS = 4
_D_GROUP = 2
_W_REGIONS = 8
_F_REGIONS = 2
_SEG_ROWS = 16
_SEG_LAT = 2
_SYNC_BATCH = 2
_D_SYNC = 64
_D_PLAN = ((3, 100), (4, 128), (5, 173), (6, 192), (7, 256))


def _dot(a, b, dims):
    return lax.dot_general(a, b, dims, preferred_element_type=_F32)


def _make_kernel(B, SK, M, H, D, DC, F):
    scale = float(D) ** -0.5
    n_hg = H // _HG
    hs = H // _HEAD_STEPS
    d_rows = SK // _D_REGIONS
    w_lat = M // _W_REGIONS
    o_rows = H * D // _W_REGIONS
    f_rows = F // _F_REGIONS
    d_lead = _D_GROUP * _D_REGIONS
    d_per_grp = d_rows // _SEG_ROWS
    d_total = B // _D_GROUP * d_per_grp
    first_c, ffn_head, ffn_tail = 4, 4 + B, 5 + B
    sem_w = ffn_head % _N_SEM
    assert _N_PACED == ffn_head - 2 and _N_SEM == 3 and 1 < _SYNC_BATCH < B - 1
    assert _D_SYNC <= (_SYNC_BATCH + 1) // _D_GROUP * d_per_grp and _D_PLAN[-1][1] == d_total
    assert all(n <= (k + 1) // _D_GROUP * d_per_grp for k, n in _D_PLAN)

    def kernel(x_hbm, ckv_hbm, wq_hbm, wuk_hbm, wuv_hbm, wo_hbm, wg_hbm, wu_hbm, wd_hbm, g_hbm,
               out_hbm, dx_hbm, dckv_hbm, dwq_hbm, dwuk_hbm, dwuv_hbm, dwo_hbm, dwg_hbm, dwu_hbm, dwd_hbm,
               x_v, g_v, c_v, d_v, wq_v, wuk_v, wuv_v, wo_v, wq_s, wuk_s, wuv_s, dwo_v,
               wg_v, wu_v, wd_v, dwg_v, dwu_v, dwd_v, out_v, dx_v,
               q_v, dctx_v, wall_v, oall_v, s_v, p_v, t_v, spin_v, sem):

        def cp(src, dst, i):
            return pltpu.make_async_copy(src, dst, sem.at[i])

        weights = {0: (wq_hbm, wq_v), 1: (wuk_hbm, wuk_v), 2: (wo_hbm, wo_v), 3: (wuv_hbm, wuv_v)}

        def part(i, lo, n):
            if i < first_c:
                src, dst = weights[i]
                if i == 2:
                    st = H // (2 * _N_PIECES)
                    sl = (pl.ds(lo * st, n * st),)
                else:
                    st = w_lat // (2 * _N_PIECES)
                    sl = (slice(None), pl.ds(lo * st, n * st))
            else:
                src, dst = ckv_hbm, c_v
                st = SK // (2 * _N_PIECES)
                sl = (i - first_c, pl.ds(pl.multiple_of(lo * st, st), n * st))
            return cp(src.at[sl], dst.at[sl], i % _N_SEM)

        def activations():
            return [cp(x_hbm, x_v, 0), cp(g_hbm, g_v, 0)]

        def r_c(b):
            return cp(ckv_hbm.at[b], c_v.at[b], (first_c + b) % _N_SEM)

        def whole(i):
            s = i % _N_SEM
            if i < first_c:
                return [cp(weights[i][0], weights[i][1], s)]
            if i < ffn_head:
                return [r_c(i - first_c)]
            hd, tail = pl.ds(0, F - _TAIL_ROWS), pl.ds(F - _TAIL_ROWS, _TAIL_ROWS)
            if i == ffn_head:
                return [cp(wg_hbm, wg_v, s), cp(wu_hbm, wu_v, s), cp(wd_hbm.at[hd], wd_v.at[hd], s)]
            return [cp(wd_hbm.at[tail], wd_v.at[tail], s)]

        def start_item(i):
            for d in ([part(i, 0, _N_PIECES)] if i < _N_PACED else whole(i)):
                d.start(priority=1)

        def wait_item(i):
            for d in whole(i):
                d.wait()

        def tick(i, j):
            part(i, _N_PIECES + j, 1).start(priority=0)

        def idle_ticks(i, j0):
            def body(j, acc):
                tick(i, j)
                return lax.fori_loop(0, _SPIN, lambda k, c: c * 1.0001 + 1.0, acc)
            if j0 < _N_PIECES:
                spin_v[...] = lax.fori_loop(j0, _N_PIECES, body, jnp.zeros((8, 128), _F32))

        def start_pieces(pairs, n, seg):
            assert n % seg == 0

            def body(j, carry):
                sl = pl.ds(pl.multiple_of(j * seg, seg), seg)
                for src, dst in pairs:
                    cp(src.at[:, sl], dst.at[:, sl], sem_w).start()
                return carry
            lax.fori_loop(0, n // seg, body, 0)

        def start_d(lo, hi):
            for k in range(lo, hi):
                lead = pl.ds(k // d_per_grp * d_lead, d_lead)
                sl = pl.ds(k % d_per_grp * _SEG_ROWS, _SEG_ROWS)
                cp(d_v.at[lead, sl], dckv_hbm.at[lead, sl], sem_w).start()

        def to_head_major(src, dst, it):
            per = w_lat // _SWAP_CH
            steps = _W_REGIONS * per // 2

            def body(i2, carry):
                tick(it, i2)
                for u in range(2):
                    i = 2 * i2 + u
                    blk = src[i // per, pl.ds(pl.multiple_of((i % per) * _SWAP_CH, _SWAP_CH), _SWAP_CH)]
                    dst[:, pl.ds(pl.multiple_of(i * _SWAP_CH, _SWAP_CH), _SWAP_CH), :] = jnp.swapaxes(blk, 0, 1)
                return carry
            lax.fori_loop(0, steps, body, 0)
            return steps

        def per_head(lhs, w_ref, dims, dst, it, j0):
            def body(i, carry):
                tick(it, j0 + i)
                sl = pl.ds(i * hs, hs)
                dst[sl] = _dot(lhs(sl), w_ref[sl], dims)
                return carry
            lax.fori_loop(0, _HEAD_STEPS, body, 0)
            return j0 + _HEAD_STEPS

        for d in activations():
            d.start(priority=0)
        for i in range(_N_SEM):
            start_item(i)

        idle_ticks(0, 0)
        for d in activations():
            d.wait()
        wait_item(0)
        start_item(_N_SEM)
        x = x_v[...].astype(_F32)
        g = g_v[...]
        xc = x - jnp.mean(x, axis=-1, keepdims=True)
        rstd = lax.rsqrt(jnp.mean(xc * xc, axis=-1, keepdims=True) + _EPS)
        xn32 = xc * rstd
        xn = xn32.astype(_BF)
        xn_h = jnp.broadcast_to(xn[None], (hs, B, M))
        g_h = jnp.broadcast_to(g[None], (hs, B, M))

        j = to_head_major(wq_v, wq_s, 1)
        idle_ticks(1, per_head(lambda sl: xn_h, wq_s, _BNN, q_v, 1, j))
        wait_item(1)
        start_item(1 + _N_SEM)
        j = to_head_major(wuk_v, wuk_s, 2)
        j = per_head(lambda sl: q_v[sl].astype(_BF), wuk_s, _BNT, t_v, 2, j)
        wall_v[:, 0:H, :] = jnp.swapaxes(t_v[...], 0, 1).astype(_BF)
        idle_ticks(2, j)
        wait_item(2)
        start_item(2 + _N_SEM)
        idle_ticks(3, per_head(lambda sl: g_h, wo_v, _BNT, dctx_v, 3, 0))
        wait_item(3)
        start_item(3 + _N_SEM)
        j = to_head_major(wuv_v, wuv_s, 4)
        j = per_head(lambda sl: dctx_v[sl].astype(_BF), wuv_s, _BNT, t_v, 4, j)
        wall_v[:, H:2 * H, :] = jnp.swapaxes(t_v[...], 0, 1).astype(_BF)
        idle_ticks(4, j)
        for i in range(5, _N_PACED):
            idle_ticks(i, 0)
            wait_item(i - 1)
            start_item(i - 1 + _N_SEM)

        def batch(b, carry):
            @pl.when(b == B - 1)
            def _():
                wait_item(ffn_head - 1)

            wb = wall_v[b]
            s_v[...] = _dot(wb, c_v[b], _NT)
            s = s_v[0:H, :]
            e = jnp.exp((s - jnp.max(s, axis=1, keepdims=True)) * scale)
            rl = 1.0 / jnp.sum(e, axis=1, keepdims=True)
            dp = s_v[H:2 * H, :]
            delta = jnp.sum(e * dp, axis=1, keepdims=True) * rl
            p = e * rl
            p_v[0:H, :] = (p * ((dp - delta) * scale)).astype(_BF)
            p_v[H:2 * H, :] = p.astype(_BF)
            p2 = p_v[...]
            oall_v[b] = _dot(p2, c_v[b], _NN)
            d_v[pl.ds(b * _D_REGIONS, _D_REGIONS)] = (
                _dot(p2, wb, _TN).astype(_BF).reshape(_D_REGIONS, d_rows, DC))

            @pl.when(b == 0)
            def _():
                wait_item(_N_PACED - 1)
                start_item(_N_PACED - 1 + _N_SEM)

            @pl.when(b == 1)
            def _():
                wait_item(_N_PACED)
                start_item(_N_PACED + _N_SEM)

            @pl.when(b == _SYNC_BATCH)
            def _():
                wait_item(ffn_head)
                start_d(0, _D_SYNC)

            lo = _D_SYNC
            for k, hi in _D_PLAN:
                @pl.when(b == k)
                def _(lo=lo, hi=hi):
                    start_d(lo, hi)
                lo = hi
            return carry

        lax.fori_loop(0, B, batch, 0)

        diag = (lax.broadcasted_iota(jnp.int32, (_HG, B * _HG), 1) % _HG
                == lax.broadcasted_iota(jnp.int32, (_HG, B * _HG), 0))

        def head_grad(a_g, y_g, dst, h0):
            at = a_g.T
            for r in range(_W_REGIONS):
                blk = at[r * w_lat:(r + 1) * w_lat]
                lhs = jnp.where(diag[None], blk[:, None, :], 0.0).astype(_BF).reshape(w_lat * _HG, B * _HG)
                dst[r, :, h0:h0 + _HG, :] = _dot(lhs, y_g, _NN).astype(_BF).reshape(w_lat, _HG, D)

        def group(y_bhd, h0):
            return y_bhd[:, h0:h0 + _HG, :].reshape(B * _HG, D).astype(_BF)

        qb = jnp.swapaxes(q_v[...], 0, 1)
        for i in range(n_hg):
            h0 = i * _HG
            head_grad(oall_v[:, h0:h0 + _HG, :].reshape(B * _HG, DC), group(qb, h0), wuk_v, h0)
        start_pieces([(wuk_v, dwuk_hbm)], w_lat, _SEG_LAT)

        db = jnp.swapaxes(dctx_v[...], 0, 1)
        for i in range(n_hg):
            h0 = i * _HG
            head_grad(oall_v[:, H + h0:H + h0 + _HG, :].reshape(B * _HG, DC), group(db, h0), wuv_v, h0)
        start_pieces([(wuv_v, dwuv_hbm)], w_lat, _SEG_LAT)

        ot = jnp.swapaxes(oall_v[...], 0, 1).astype(_BF)
        ctx = _dot(ot[H:2 * H], wuv_s[...], _BNN).astype(_BF)
        attn = jnp.sum(_dot(ctx, wo_v[...], _BNN), axis=0)
        ctx2 = jnp.swapaxes(ctx, 0, 1).reshape(B, H * D)
        dwo_v[...] = _dot(ctx2, g, _TN).astype(_BF).reshape(_W_REGIONS, o_rows, M)
        start_pieces([(dwo_v, dwo_hbm)], o_rows, _SEG_ROWS)

        dq = _dot(ot[0:H], wuk_s[...], _BNN)
        dxn_attn = jnp.sum(_dot(dq.astype(_BF), wq_s[...], _BNT), axis=0)
        dqb = jnp.swapaxes(dq, 0, 1)
        xn_rep = jnp.broadcast_to(xn.astype(_F32)[:, None, :], (B, _HG, M)).reshape(B * _HG, M)
        for i in range(n_hg):
            head_grad(xn_rep, group(dqb, i * _HG), wq_v, i * _HG)
        start_pieces([(wq_v, dwq_hbm)], w_lat, _SEG_LAT)

        wait_item(ffn_tail)
        a = _dot(xn, wg_v[...], _NT)
        u = _dot(xn, wu_v[...], _NT)
        k0, k1 = math.sqrt(2.0 / math.pi), 0.044715
        th = jnp.tanh(k0 * (a + k1 * a * a * a))
        gelu = 0.5 * a * (1.0 + th)
        dgelu = 0.5 * (1.0 + th) + 0.5 * a * (1.0 - th * th) * (k0 * (1.0 + 3.0 * k1 * a * a))
        hh = (gelu * u).astype(_BF)
        ffn = _dot(hh, wd_v[...], _NN)
        dh = _dot(g, wd_v[...], _NT)
        da = (dh * u * dgelu).astype(_BF)
        du = (dh * gelu).astype(_BF)
        out_v[...] = (x + attn + ffn).astype(_BF)
        cp(out_v, out_hbm, sem_w).start()
        dxn = dxn_attn + _dot(da, wg_v[...], _NN) + _dot(du, wu_v[...], _NN)
        m1 = jnp.mean(dxn, axis=-1, keepdims=True)
        m2 = jnp.mean(dxn * xn32, axis=-1, keepdims=True)
        dx_v[...] = (g.astype(_F32) + rstd * (dxn - m1 - xn32 * m2)).astype(_BF)
        cp(dx_v, dx_hbm, sem_w).start()
        dwg_v[...] = _dot(da, xn, _TN).astype(_BF).reshape(_F_REGIONS, f_rows, M)
        dwu_v[...] = _dot(du, xn, _TN).astype(_BF).reshape(_F_REGIONS, f_rows, M)
        dwd_v[...] = _dot(hh, g, _TN).astype(_BF).reshape(_F_REGIONS, f_rows, M)
        start_pieces([(dwg_v, dwg_hbm), (dwu_v, dwu_hbm), (dwd_v, dwd_hbm)], f_rows, _SEG_ROWS)

        for src, dst in ((d_v, dckv_hbm), (wuk_v, dwuk_hbm), (wuv_v, dwuv_hbm), (dwo_v, dwo_hbm),
                         (wq_v, dwq_hbm), (out_v, out_hbm), (dx_v, dx_hbm), (dwg_v, dwg_hbm),
                         (dwu_v, dwu_hbm), (dwd_v, dwd_hbm)):
            cp(src, dst, sem_w).wait()

    return kernel


@jax.jit
def pallas_parallel_sum__compressed_kv_cla__geglu_ffn__decode_kernel(
    A_x, A_c_kv, A_w_q, A_w_uk, A_w_uv, A_w_o, B_x, B_w_gate, B_w_up, B_w_down, grad_out,
):
    del B_x
    B, _, M = A_x.shape
    SK, DC = A_c_kv.shape[1:]
    H, D = A_w_q.shape[1:]
    F = B_w_gate.shape[1]
    assert DC == M and H % _HG == 0
    bf = _BF

    w4 = (_W_REGIONS, M // _W_REGIONS, H, D)
    d3 = (B * _D_REGIONS, SK // _D_REGIONS, DC)
    o3 = (_W_REGIONS, H * D // _W_REGIONS, M)
    f3 = (_F_REGIONS, F // _F_REGIONS, M)
    ins = (A_x.reshape(B, M), A_c_kv, A_w_q.reshape(w4), A_w_uk.reshape(w4), A_w_uv.reshape(w4), A_w_o,
           B_w_gate.T, B_w_up.T, B_w_down, grad_out.reshape(B, M))
    out_shapes = ((B, M), (B, M), d3, w4, w4, w4, o3, f3, f3, f3)

    hbm = pl.BlockSpec(memory_space=pl.ANY)
    vmem = pltpu.VMEM
    scratch = [
        vmem((B, M), bf), vmem((B, M), bf),
        vmem((B, SK, DC), bf), vmem(d3, bf),
        vmem(w4, bf), vmem(w4, bf), vmem(w4, bf), vmem((H, D, M), bf),
        vmem((H, M, D), bf), vmem((H, DC, D), bf), vmem((H, DC, D), bf),
        vmem(o3, bf),
        vmem((F, M), bf), vmem((F, M), bf), vmem((F, M), bf),
        vmem(f3, bf), vmem(f3, bf), vmem(f3, bf),
        vmem((B, M), bf), vmem((B, M), bf),
        vmem((H, B, D), _F32), vmem((H, B, D), _F32),
        vmem((B, 2 * H, DC), bf), vmem((B, 2 * H, DC), _F32),
        vmem((2 * H, SK), _F32), vmem((2 * H, SK), bf),
        vmem((H, B, DC), _F32), vmem((8, 128), _F32),
        pltpu.SemaphoreType.DMA((_N_SEM,)),
    ]
    out, dx, dckv, dwq, dwuk, dwuv, dwo, dwg_t, dwu_t, dwd = pl.pallas_call(
        _make_kernel(B, SK, M, H, D, DC, F),
        out_shape=tuple(jax.ShapeDtypeStruct(s, bf) for s in out_shapes),
        in_specs=[hbm] * len(ins),
        out_specs=tuple([hbm] * len(out_shapes)),
        scratch_shapes=scratch,
        compiler_params=pltpu.CompilerParams(vmem_limit_bytes=120 * 1024 * 1024),
        name="mla_ffn_fwd_bwd",
    )(*ins)
    return (out.reshape(B, 1, M), dx.reshape(B, 1, M), dckv.reshape(B, SK, DC), dwq.reshape(M, H, D),
            dwuk.reshape(DC, H, D), dwuv.reshape(DC, H, D), dwo.reshape(H, D, M),
            dwg_t.reshape(F, M).T, dwu_t.reshape(F, M).T, dwd.reshape(F, M))
```
